```python
import jax
import jax.numpy as jnp

def _softmax(x, axis=-1):
    return jax.nn.softmax(x, axis=axis)
def _gelu(x):
    return jax.nn.gelu(x, approximate=True)
def _silu(x):
    return jax.nn.silu(x)
def _sigmoid(x):
    return jax.nn.sigmoid(x)
def _layernorm(x, axis=-1, eps=1e-5):
    m = jnp.mean(x, axis=axis, keepdims=True)
    v = jnp.var(x, axis=axis, keepdims=True)
    return (x - m) / jnp.sqrt(v + eps)
def _scatter_add(tgt, idx, src, axis=0):
    return tgt.at[idx].add(src)
def _segment_sum(src, seg, n):
    return jax.ops.segment_sum(src, seg, n)
class _Rng:
    def __init__(self, key):
        self._k = key
    def _next(self):
        self._k, sub = jax.random.split(self._k)
        return sub
    def normal(self, shape):
        return jax.random.normal(self._next(), shape, dtype=jnp.bfloat16)
    def randint(self, lo, hi, shape):
        return jax.random.randint(self._next(), shape, lo, hi, dtype=jnp.int32)
    def uniform(self, shape, lo=0.0, hi=1.0):
        return jax.random.uniform(self._next(), shape, jnp.bfloat16, lo, hi)
    def permutation(self, n):
        return jax.random.permutation(self._next(), n)


kernel_name = 'parallel_sum__compressed_kv_cla__moe_arch_mod__prompt'

def setup_inputs():
    _rng = _Rng(jax.random.key(int.from_bytes(__import__("os").urandom(4), "little")))
    _w = (lambda a: (lambda t: t.astype(jnp.bfloat16) if jnp.issubdtype(t.dtype, jnp.floating) else t)(jnp.asarray(a)))
    def _A_setup():
        B, H, Sq, Sk, D, M = 1, 32, 2048, 2048, 128, 640
        Dc = 4 * D
        return {
            "x": _w((lambda *s: _rng.normal(s) * 0.05)(B, Sq, M)),
            "c_kv": _w((lambda *s: _rng.normal(s) * 0.05)(B, Sk, Dc)),
            "w_q": _w((lambda *s: _rng.normal(s) * 0.05)(M, H, D) * (M ** -0.5)),
            "w_uk": _w((lambda *s: _rng.normal(s) * 0.05)(Dc, H, D) * (Dc ** -0.5)),
            "w_uv": _w((lambda *s: _rng.normal(s) * 0.05)(Dc, H, D) * (Dc ** -0.5)),
            "w_o": _w((lambda *s: _rng.normal(s) * 0.05)(H, D, M) * ((H * D) ** -0.5)),
        }
    _A_in = _A_setup()

    def _B_setup():
        B, S, D, F, C = 1, 2048, 640, 1728, 8
        return {
            "x": _w((lambda *s: _rng.normal(s) * 0.05)(B, S, D)),
            "w_r": _w((lambda *s: _rng.normal(s) * 0.05)(D)),
            "w_gate": _w((lambda *s: _rng.normal(s) * 0.05)(D, F)),
            "w_up": _w((lambda *s: _rng.normal(s) * 0.05)(D, F)),
            "w_down": _w((lambda *s: _rng.normal(s) * 0.05)(F, D)),
        }
    _B_in = _B_setup()

    return {
        "A_x": _A_in["x"],
        "A_c_kv": _A_in["c_kv"],
        "A_w_q": _A_in["w_q"],
        "A_w_uk": _A_in["w_uk"],
        "A_w_uv": _A_in["w_uv"],
        "A_w_o": _A_in["w_o"],
        "B_x": _B_in["x"],
        "B_w_r": _B_in["w_r"],
        "B_w_gate": _B_in["w_gate"],
        "B_w_up": _B_in["w_up"],
        "B_w_down": _B_in["w_down"],
    }

def reference(A_x, A_c_kv, A_w_q, A_w_uk, A_w_uv, A_w_o, B_x, B_w_r, B_w_gate, B_w_up, B_w_down):
    def _A_ref(x, c_kv, w_q, w_uk, w_uv, w_o):
        B, Sq, M = x.shape[0], x.shape[1], x.shape[2]
        Sk = c_kv.shape[1]
        H, D = w_q.shape[1], w_q.shape[2]
        q = jnp.einsum("bqm,mhd->bhqd", x, w_q)
        k = jnp.einsum("bkc,chd->bhkd", c_kv, w_uk)
        v = jnp.einsum("bkc,chd->bhkd", c_kv, w_uv)
        scores = jnp.einsum("bhqd,bhkd->bhqk", q, k) * (D ** -0.5)
        off = Sk - Sq
        qi = jnp.arange(Sq)[:, None]
        kj = jnp.arange(Sk)[None, :]
        cmask = kj <= (qi + off)
        scores = jnp.where(cmask[None, None], scores, -1e9)
        p = _softmax(scores, axis=-1)
        ctx = jnp.einsum("bhqk,bhkd->bhqd", p, v)
        return jnp.einsum("bhqd,hdm->bqm", ctx, w_o)

    def _B_ref(x, w_r, w_gate, w_up, w_down):
        B, S, D = x.shape
        C = 8
        r = x @ w_r
        idx = jnp.argsort(-r, axis=-1)[:, :C]
        idx_e = jnp.repeat(idx.reshape(B, C, 1), D, axis=2)
        x_sel = jnp.take_along_axis(x, idx_e, axis=1)
        g = _silu(x_sel @ w_gate)
        u = x_sel @ w_up
        y = (g * u) @ w_down
        r_sel = _sigmoid(jnp.take_along_axis(r, idx, axis=1))
        y = y * r_sel.reshape(B, C, 1)
        b_off = (jnp.arange(B) * S).reshape(B, 1)
        flat_idx = (idx + b_off).reshape(B * C)
        zero = (x * 0.0).reshape(B * S, D)
        upd = _scatter_add(zero, flat_idx, y.reshape(B * C, D), axis=0)
        return x + upd.reshape(B, S, D)

    x = A_x
    xn = _layernorm(x, axis=-1)
    return x + _A_ref(xn, A_c_kv, A_w_q, A_w_uk, A_w_uv, A_w_o) + _B_ref(xn, B_w_r, B_w_gate, B_w_up, B_w_down)
```

```python
import functools
import jax
import jax.numpy as jnp
import numpy as np
from jax import lax
import jax.experimental.pallas as pl
import jax.experimental.pallas.tpu as pltpu

S, M, DC, H, D, F, C = 2048, 640, 512, 32, 128, 1728, 8
HG = 8
NG = H // HG
LOG2E = 1.4426950408889634
QSCALE = float(D ** -0.5) * LOG2E
NEG = -1e30
BF = jnp.bfloat16
F32 = jnp.float32

def _rb(v):
    return v.astype(BF).astype(F32)

def _dot(a, b):
    return jnp.dot(a, b, preferred_element_type=F32)

def _dot_nt(a, b):
    return lax.dot_general(a, b, (((1,), (1,)), ((), ())), preferred_element_type=F32)

def _attn_head(h, q_s, k_s, v_s, ctx_s, BQ):
    nb = S // BQ
    row = lax.broadcasted_iota(jnp.int32, (BQ, BQ), 0)
    col = lax.broadcasted_iota(jnp.int32, (BQ, BQ), 1)
    tri = col <= row
    def qk(i):
        q = q_s[h, i * BQ:(i + 1) * BQ, :]
        k = k_s[h, 0:(i + 1) * BQ, :]
        return _dot_nt(q, k)
    def sm(i, s):
        if i > 0:
            sd = jnp.where(tri, s[:, i * BQ:], NEG)
            s = jnp.concatenate([s[:, :i * BQ], sd], axis=1)
        else:
            s = jnp.where(tri, s, NEG)
        m = jnp.max(s, axis=1, keepdims=True)
        p = jnp.exp2(s - m)
        l = jnp.sum(p, axis=1, keepdims=True)
        return p.astype(BF), l
    def pv(i, p, l):
        v = v_s[h, 0:(i + 1) * BQ, :]
        o = _dot(p, v)
        ctx_s[h, i * BQ:(i + 1) * BQ, :] = (o / l).astype(BF)
    s_next = qk(0)
    for i in range(nb):
        s = s_next
        if i + 1 < nb:
            s_next = qk(i + 1)
        p, l = sm(i, s)
        pv(i, p, l)

def kernel(x_ref, c_ref, wq_ref, wuk_ref, wuv_ref, wo_ref, wr_ref, wg_hbm, wu_hbm, wd_hbm, o_ref,
           xn_s, acc_s, wq_s, wk_s, wv_s, q_s, k_s, v_s, ctx_s, wg_s, wu_s, wd_s, sems, *, BQ):
    g = pl.program_id(0)
    RB = 256
    cps = [pltpu.make_async_copy(wg_hbm, wg_s, sems.at[0]),
           pltpu.make_async_copy(wu_hbm, wu_s, sems.at[1]),
           pltpu.make_async_copy(wd_hbm, wd_s, sems.at[2])]

    @pl.when(g == 0)
    def _():
        for cp in cps:
            cp.start()
        def ln(r, carry):
            rows = pl.ds(pl.multiple_of(r * RB, RB), RB)
            x = x_ref[rows, :].astype(F32)
            mean = jnp.sum(x, axis=1, keepdims=True) / M
            cen = x - mean
            var = jnp.sum(cen * cen, axis=1, keepdims=True) / M
            d = _rb(x - _rb(mean))
            den = _rb(jnp.sqrt(_rb(_rb(var) + float(np.asarray(1e-5, dtype=BF)))))
            xn = (d / den).astype(BF)
            xn_s[rows, :] = xn
            acc_s[rows, :] = x + xn.astype(F32)
            return carry
        lax.fori_loop(0, S // RB, ln, 0)

    wq_s[...] = wq_ref[...].reshape(M, HG * D)
    wk_s[...] = wuk_ref[...].reshape(DC, HG * D)
    wv_s[...] = wuv_ref[...].reshape(DC, HG * D)

    PB = 512
    def proj(r, carry):
        rows = pl.ds(pl.multiple_of(r * PB, PB), PB)
        q = (_dot(xn_s[rows, :], wq_s[...]) * QSCALE).astype(BF)
        for h in range(HG):
            q_s[h, rows, :] = q[:, h * D:(h + 1) * D]
        c = c_ref[rows, :]
        k = _dot(c, wk_s[...]).astype(BF)
        for h in range(HG):
            k_s[h, rows, :] = k[:, h * D:(h + 1) * D]
        v = _dot(c, wv_s[...]).astype(BF)
        for h in range(HG):
            v_s[h, rows, :] = v[:, h * D:(h + 1) * D]
        return carry
    lax.fori_loop(0, S // PB, proj, 0)

    def att(h, carry):
        _attn_head(h, q_s, k_s, v_s, ctx_s, BQ)
        return carry
    lax.fori_loop(0, HG, att, 0)

    def oproj(r, carry):
        rows = pl.ds(pl.multiple_of(r * PB, PB), PB)
        ctx = jnp.concatenate([ctx_s[h, rows, :] for h in range(HG)], axis=1)
        acc_s[rows, :] += _dot(ctx, wo_ref[...])
        return carry
    lax.fori_loop(0, S // PB, oproj, 0)

    @pl.when(g == NG - 1)
    def _():
        for cp in cps:
            cp.wait()
        wr = jnp.broadcast_to(wr_ref[...].reshape(1, M), (16, M))
        r = _rb(_dot_nt(wr, xn_s[...]))[:8]
        tok = lax.broadcasted_iota(jnp.int32, (8, S), 1)
        slot = lax.broadcasted_iota(jnp.int32, (8, S), 0)
        slot1 = lax.broadcasted_iota(jnp.int32, (8, 1), 0)
        taken = jnp.zeros((8, S), jnp.bool_)
        onehot = jnp.zeros((8, S), F32)
        rsel = jnp.zeros((8, 1), F32)
        cur = r
        for j in range(C):
            mx = jnp.max(cur, axis=1, keepdims=True)
            idx = jnp.min(jnp.where(cur == mx, tok, S), axis=1, keepdims=True)
            hit = tok == idx
            onehot = jnp.where(jnp.logical_and(hit, slot == j), 1.0, onehot)
            rsel = jnp.where(slot1 == j, mx, rsel)
            cur = jnp.where(hit, -jnp.inf, cur)
        oh = jnp.concatenate([onehot, jnp.zeros((8, S), F32)], axis=0).astype(BF)
        xs = _dot(oh, xn_s[...]).astype(BF)
        gt = _dot_nt(xs, wg_s[...])
        up = _dot_nt(xs, wu_s[...])
        hh = (gt * jax.nn.sigmoid(gt) * up).astype(BF)
        y = _dot(hh, wd_s[...])[:8] * jax.nn.sigmoid(rsel)
        y16 = jnp.concatenate([y, jnp.zeros((8, M), F32)], axis=0).astype(BF)
        upd = lax.dot_general(oh, y16, (((0,), (0,)), ((), ())), preferred_element_type=F32)
        o_ref[...] = (acc_s[...] + upd).astype(BF)


def _make(BQ=128):
    def fn(A_x, A_c_kv, A_w_q, A_w_uk, A_w_uv, A_w_o, B_x, B_w_r, B_w_gate, B_w_up, B_w_down):
        x = A_x.reshape(S, M)
        c = A_c_kv.reshape(S, DC)
        wo = A_w_o.reshape(H * D, M)
        out = pl.pallas_call(
            functools.partial(kernel, BQ=BQ),
            grid=(NG,),
            in_specs=[
                pl.BlockSpec((S, M), lambda g: (0, 0)),
                pl.BlockSpec((S, DC), lambda g: (0, 0)),
                pl.BlockSpec((M, HG, D), lambda g: (0, g, 0)),
                pl.BlockSpec((DC, HG, D), lambda g: (0, g, 0)),
                pl.BlockSpec((DC, HG, D), lambda g: (0, g, 0)),
                pl.BlockSpec((HG * D, M), lambda g: (g, 0)),
                pl.BlockSpec((M,), lambda g: (0,)),
                pl.BlockSpec(memory_space=pltpu.HBM),
                pl.BlockSpec(memory_space=pltpu.HBM),
                pl.BlockSpec(memory_space=pltpu.HBM),
            ],
            out_specs=pl.BlockSpec((S, M), lambda g: (0, 0)),
            out_shape=jax.ShapeDtypeStruct((S, M), BF),
            scratch_shapes=[
                pltpu.VMEM((S, M), BF), pltpu.VMEM((S, M), F32),
                pltpu.VMEM((M, HG * D), BF), pltpu.VMEM((DC, HG * D), BF), pltpu.VMEM((DC, HG * D), BF),
                pltpu.VMEM((HG, S, D), BF), pltpu.VMEM((HG, S, D), BF), pltpu.VMEM((HG, S, D), BF),
                pltpu.VMEM((HG, S, D), BF),
                pltpu.VMEM((F, M), BF), pltpu.VMEM((F, M), BF), pltpu.VMEM((F, M), BF),
                pltpu.SemaphoreType.DMA((3,)),
            ],
            compiler_params=pltpu.CompilerParams(
                dimension_semantics=("arbitrary",), vmem_limit_bytes=110 * 1024 * 1024),
        )(x, c, A_w_q, A_w_uk, A_w_uv, wo, B_w_r, B_w_gate.T, B_w_up.T, B_w_down)
        return out.reshape(1, S, M)
    return fn


_impl = _make()


@jax.jit
def pallas_parallel_sum__compressed_kv_cla__moe_arch_mod__prompt_kernel(
    A_x, A_c_kv, A_w_q, A_w_uk, A_w_uv, A_w_o, B_x, B_w_r, B_w_gate, B_w_up, B_w_down,
):
    return _impl(A_x, A_c_kv, A_w_q, A_w_uk, A_w_uv, A_w_o, B_x, B_w_r, B_w_gate, B_w_up, B_w_down)
```

```python
import jax
import jax.numpy as jnp
import numpy as np
from jax import lax
import jax.experimental.pallas as pl
import jax.experimental.pallas.tpu as pltpu

S, M, DC, H, D, F, C = 2048, 640, 512, 32, 128, 1728, 8
NP = H // 2
BQ = 128
RB = 2 * BQ
NR = S // RB
KH = 256
AHEAD = 4
QSCALE = float(D ** -0.5) * 1.4426950408889634
EPS_BF = float(np.asarray(1e-5, dtype=jnp.bfloat16))
NEG = -1e30
BF = jnp.bfloat16
F32 = jnp.float32
I32 = jnp.int32
U32 = jnp.uint32


def _rb(v):
    return v.astype(BF).astype(F32)


def _dot(a, b):
    return jnp.dot(a, b, preferred_element_type=F32)


def _dot_nt(a, b):
    return lax.dot_general(a, b, (((1,), (1,)), ((), ())), preferred_element_type=F32)


def _ds(start, size, align):
    if isinstance(start, int):
        return pl.ds(start, size)
    return pl.ds(pl.multiple_of(start, align), size)


def _left7(a11, a12, a21, a22):
    return [a11 + a22, a21 + a22, a11, a22, a11 + a12, a21 - a11, a12 - a22]


def _right7(b11, b12, b21, b22):
    return [b11 + b22, b11, b12 - b22, b21 - b11, b22, b11 + b12, b21 + b22]


def _block_matmul(a, b):
    def m(i):
        return _dot(a(i), b(i))

    m4 = m(3)
    m3 = m(2)
    m1 = m(0)
    c11 = m1 + m4
    c22 = m1 + m3
    m2 = m(1)
    c21 = m2 + m4
    c22 = c22 - m2
    m5 = m(4)
    c12 = m3 + m5
    c11 = c11 - m5
    c22 = c22 + m(5)
    c11 = c11 + m(6)
    return c11, c12, c21, c22


def _attention(q_s, k_s, v_s, lag, fill):
    nb = S // BQ
    look = 2
    row = lax.broadcasted_iota(I32, (BQ, BQ), 0)
    col = lax.broadcasted_iota(I32, (BQ, BQ), 1)
    tri = col <= row
    sums = []

    def qk(h, i):
        return _dot_nt(q_s[h, i * BQ:(i + 1) * BQ, :], k_s[h, 0:(i + 1) * BQ, :])

    def softmax_pv(h, i, s):
        sd = jnp.where(tri, s[:, i * BQ:], NEG)
        s = jnp.concatenate([s[:, :i * BQ], sd], axis=1) if i > 0 else sd
        m = jnp.max(s, axis=1, keepdims=True)
        if len(sums) >= lag:
            old = sums.pop(0)
            m = jnp.where(old < 0.0, old, m)
        p = jnp.exp2(s - m)
        l = jnp.sum(p, axis=1, keepdims=True)
        sums.append(l)
        o = _dot(p.astype(BF), v_s[h, 0:(i + 1) * BQ, :])
        r = pl.reciprocal(l, approx=True)
        r = r * (2.0 - l * r)
        return o * r

    order = list(range(0, nb, 2)) + list(range(nb - 1, 0, -2))
    items = [(h, i) for h in range(2) for i in order]
    scores, ctx = {}, {}
    for t in range(look):
        scores[t] = qk(*items[t])
    for t, it in enumerate(items):
        if t + look < len(items):
            scores[t + look] = qk(*items[t + look])
        fill(t)
        ctx[it] = softmax_pv(*it, scores.pop(t))
    return ctx


def _kernel(x_hbm, c_hbm, wq_hbm, wk_hbm, wv_hbm, wo_hbm, wr_ref, wg_hbm, wu_hbm, wd_hbm, o_hbm,
            x_s, c_s, xn_s, acc_s, xa_s, ca_s, wq3, wk3, wv3, wo_s, wq_s, wqt_s, wkv_s, q_s, k_s, v_s,
            wg_s, wu_s, wd_s, r_s, sem_x, sem_c, sem_w, sem_f, sem_o):

    w3 = [(wk_hbm.bitcast(U32), wk3), (wv_hbm.bitcast(U32), wv3), (wq_hbm.bitcast(U32), wq3)]

    def w_copies(k, lo, hi):
        return [pltpu.make_async_copy(src.at[:, lo:hi, :], dst.at[lo // 8, :, lo % 8:lo % 8 + hi - lo, :],
                                      sem_w.at[3 * k + i])
                for i, (src, dst) in enumerate(w3)]

    w_first, w_a, w_b, w_c = w_copies(0, 0, 1), w_copies(1, 1, 4), w_copies(2, 4, 8), w_copies(3, 8, 16)
    wo_first = pltpu.make_async_copy(wo_hbm.at[0:2 * D, :], wo_s.at[0:2 * D, :], sem_f.at[3])
    wo_rest = pltpu.make_async_copy(wo_hbm.at[2 * D:H * D, :], wo_s.at[2 * D:H * D, :], sem_f.at[4])
    f_copies = [pltpu.make_async_copy(wg_hbm, wg_s, sem_f.at[0]),
                pltpu.make_async_copy(wu_hbm, wu_s, sem_f.at[1]),
                pltpu.make_async_copy(wd_hbm, wd_s, sem_f.at[2])]

    def in_copies(r):
        rows = _ds(r * RB, RB, RB)
        return [pltpu.make_async_copy(c_hbm.at[rows, :], c_s.at[rows, :], sem_c.at[r]),
                pltpu.make_async_copy(x_hbm.at[rows, :], x_s.at[rows, :], sem_x.at[r])]

    def start(copies):
        for cp in copies:
            cp.start()

    def wait(copies):
        for cp in copies:
            cp.wait()

    def pick(w, p):
        n = w.shape[1]
        u = w.reshape(2 * n * 8, D)[pl.ds((p // 8) * (n * 8) + p % 8, n, stride=8), :]
        return pltpu.bitcast(u << 16, F32), pltpu.bitcast((u >> 16) << 16, F32)

    def load_wkv(p):
        wk = jnp.concatenate(pick(wk3, p), axis=1)
        wv = jnp.concatenate(pick(wv3, p), axis=1)
        for i, b in enumerate(_right7(wk[:KH], wv[:KH], wk[KH:], wv[KH:])):
            wkv_s[i] = b.astype(BF)

    def load_wq(p):
        h0, h1 = pick(wq3, p)
        for i, b in enumerate(_right7(h0[:KH], h1[:KH], h0[KH:2 * KH], h1[KH:2 * KH])):
            wq_s[i] = b.astype(BF)
        wqt_s[...] = jnp.concatenate([h0[2 * KH:], h1[2 * KH:]], axis=1).astype(BF)

    def kv_proj(r, n, direct=None):
        rows = _ds(r * BQ, n * BQ, BQ)
        c4 = _block_matmul(lambda i: direct[i] if direct and i in direct else ca_s[i, rows, :],
                           lambda i: wkv_s[i])
        for t in range(n):
            for u in range(2):
                dst = _ds((r + t) * RB + u * BQ, BQ, BQ)
                for h in range(2):
                    k_s[h, dst, :] = c4[2 * u][t * BQ:(t + 1) * BQ, h * D:(h + 1) * D].astype(BF)
                    v_s[h, dst, :] = c4[2 * u + 1][t * BQ:(t + 1) * BQ, h * D:(h + 1) * D].astype(BF)

    def q_proj(r, n):
        rows = _ds(r * BQ, n * BQ, BQ)
        c4 = _block_matmul(lambda i: xa_s[i, rows, :], lambda i: wq_s[i])
        rest = _dot(xn_s[_ds(r * RB, n * RB, RB), 2 * KH:], wqt_s[...])
        for t in range(n):
            for u in range(2):
                dst = _ds((r + t) * RB + u * BQ, BQ, BQ)
                lo = t * RB + u * BQ
                for h in range(2):
                    q = c4[2 * u + h][t * BQ:(t + 1) * BQ] + rest[lo:lo + BQ, h * D:(h + 1) * D]
                    q_s[h, dst, :] = (q * QSCALE).astype(BF)

    def o_proj(p, ctx, n, emit):
        wo = wo_s[_ds(p * 2 * D, 2 * D, 2 * D), :]
        wf = wo.astype(F32)
        b7 = [b.astype(BF) for b in _right7(wf[:D, :KH], wf[:D, KH:2 * KH], wf[D:, :KH], wf[D:, KH:2 * KH])]
        for r in range(0, NR, n):
            full = jnp.concatenate(
                [jnp.concatenate([ctx[0, i], ctx[1, i]], axis=1).astype(BF) for i in range(2 * r, 2 * (r + n))],
                axis=0)
            a7 = [_left7(ctx[0, 2 * t], ctx[1, 2 * t], ctx[0, 2 * t + 1], ctx[1, 2 * t + 1])
                  for t in range(r, r + n)]
            c4 = _block_matmul(lambda i: jnp.concatenate([a[i].astype(BF) for a in a7], axis=0),
                               lambda i: b7[i])
            rest = _dot(full, wo[:, 2 * KH:])
            left = jnp.concatenate(
                [jnp.concatenate([c4[2 * u][t * BQ:(t + 1) * BQ], c4[2 * u + 1][t * BQ:(t + 1) * BQ]], axis=1)
                 for t in range(n) for u in range(2)], axis=0)
            emit(r, jnp.concatenate([left, rest], axis=1))

    start(w_first[:2])
    start(in_copies(0))
    start(w_first[2:])
    wait(w_first)
    for r in range(1, AHEAD):
        start(in_copies(r))
    load_wkv(0)
    load_wq(0)

    def prologue(r, carry):
        @pl.when(r + AHEAD < NR)
        def _():
            start(in_copies(jnp.minimum(r + AHEAD, NR - 1)))

        @pl.when(r == NR - AHEAD - 1)
        def _():
            start(w_a + [wo_first])

        wait(in_copies(r))
        rows, half = _ds(r * RB, RB, RB), _ds(r * BQ, BQ, BQ)
        cb = c_s[rows, :]
        c = cb.astype(F32)
        for i, a in enumerate(_left7(c[:BQ, :KH], c[:BQ, KH:], c[BQ:, :KH], c[BQ:, KH:])):
            ca_s[i, half, :] = a.astype(BF)
        kv_proj(r, 1, {2: cb[:BQ, :KH], 3: cb[BQ:, KH:]})

        x = x_s[rows, :].astype(F32)
        mean = jnp.sum(x, axis=1, keepdims=True) / M
        cen = x - mean
        var = jnp.sum(cen * cen, axis=1, keepdims=True) / M
        den = _rb(jnp.sqrt(_rb(_rb(var) + EPS_BF)))
        xn = (_rb(x - _rb(mean)) * (1.0 / den)).astype(BF)
        xn_s[rows, :] = xn
        xf = xn.astype(F32)
        acc_s[rows, :] = x + xf
        for i, a in enumerate(_left7(xf[:BQ, :KH], xf[:BQ, KH:2 * KH], xf[BQ:, :KH], xf[BQ:, KH:2 * KH])):
            xa_s[i, half, :] = a.astype(BF)

        sc = jnp.sum(xf * wr_ref[...].reshape(1, M).astype(F32), axis=1, keepdims=True)
        lane = lax.broadcasted_iota(I32, (8, 128), 1)
        dense = jnp.full((8, 128), -jnp.inf, F32)
        for i in range(RB // 8):
            dense = jnp.where(lane == i, sc[i * 8:(i + 1) * 8, :], dense)
        r_s[r] = dense
        q_proj(r, 1)
        return carry

    lax.fori_loop(0, NR, prologue, 0)
    wait(w_a)
    start(w_b + [wo_rest])
    load_wq(1)
    wait([wo_first])

    def accumulate(r, out):
        acc_s[r * RB:r * RB + out.shape[0], :] += out

    def body(p, carry):
        @pl.when(p == 1)
        def _():
            wait(w_b + [wo_rest])
            start(w_c + f_copies)

        @pl.when(p == 4)
        def _():
            wait(w_c + f_copies)

        ctx = _attention(q_s, k_s, v_s, 10, lambda t: None)
        for r in range(0, NR, 4):
            q_proj(r, 4)
        load_wq(jnp.minimum(p + 2, NP - 1))
        load_wkv(p + 1)
        for r in range(0, NR, 2):
            kv_proj(r, 2)
        o_proj(p, ctx, 4, accumulate)
        return carry

    lax.fori_loop(0, NP - 1, body, 0)

    shp = (NR * 8, 128)
    sc = _rb(r_s[...].reshape(shp))
    sc = jnp.where(sc != sc, -jnp.inf, sc)
    sub = lax.broadcasted_iota(I32, shp, 0)
    lane = lax.broadcasted_iota(I32, shp, 1)
    tok = jnp.where(lane < RB // 8, (sub // 8) * RB + lane * 8 + sub % 8, S)
    slot = lax.broadcasted_iota(I32, (C, 1), 0)
    row16 = lax.broadcasted_iota(I32, (16, 1), 0)
    xsel = jnp.zeros((C, M), F32)
    rsel = jnp.zeros((C, 1), F32)
    idxs = []
    for j in range(C):
        mx = jnp.max(sc)
        idx = jnp.min(jnp.where(sc == mx, tok, S))
        hit = tok == idx
        sc = jnp.where(hit, -jnp.inf, sc)
        tok = jnp.where(hit, S, tok)
        idx = jnp.clip(idx, 0, S - 1)
        idxs.append(idx)
        blk = xn_s[_ds((idx // 16) * 16, 16, 16), :].astype(F32)
        xrow = jnp.sum(jnp.where(row16 == idx % 16, blk, 0.0), axis=0, keepdims=True)
        xsel = jnp.where(slot == j, xrow, xsel)
        rsel = jnp.where(slot == j, mx, rsel)
    xs = jnp.concatenate([xsel, jnp.zeros((16 - C, M), F32)], axis=0).astype(BF)

    nf = pl.cdiv(F, D)
    first = 8
    st = {"y": None}

    def ffn(t):
        j, second = divmod(t - first, 2)
        if not 0 <= j <= nf:
            return
        cols = slice(j * D, min((j + 1) * D, F))
        if not second:
            if j < nf:
                st["g"] = _dot_nt(xs, wg_s[cols, :])
            if j > 0:
                part = _dot(st.pop("h"), wd_s[(j - 1) * D:min(j * D, F), :])
                st["y"] = part if st["y"] is None else st["y"] + part
        elif j < nf:
            g = st.pop("g")
            st["h"] = (g * jax.nn.sigmoid(g) * _dot_nt(xs, wu_s[cols, :])).astype(BF)

    ctx = _attention(q_s, k_s, v_s, 11, ffn)
    for t in range(len(ctx), first + 2 * nf + 1):
        ffn(t)
    y = st["y"][:C] * jax.nn.sigmoid(rsel)
    for j in range(C):
        rows = _ds((idxs[j] // 8) * 8, 8, 8)
        acc_s[rows, :] += jnp.where(slot == idxs[j] % 8, y[j:j + 1, :], 0.0)

    outs = []

    def emit(r, out):
        rows = pl.ds(r * RB, RB)
        x_s[rows, :] = (acc_s[rows, :] + out).astype(BF)
        outs.append(pltpu.make_async_copy(x_s.at[rows, :], o_hbm.at[rows, :], sem_o.at[r]))
        outs[-1].start()

    o_proj(NP - 1, ctx, 1, emit)
    wait(outs)


@jax.jit
def pallas_parallel_sum__compressed_kv_cla__moe_arch_mod__prompt_kernel(
    A_x: jax.Array,
    A_c_kv: jax.Array,
    A_w_q: jax.Array,
    A_w_uk: jax.Array,
    A_w_uv: jax.Array,
    A_w_o: jax.Array,
    B_x: jax.Array,
    B_w_r: jax.Array,
    B_w_gate: jax.Array,
    B_w_up: jax.Array,
    B_w_down: jax.Array,
):
    del B_x
    hbm = pl.BlockSpec(memory_space=pltpu.HBM)
    out = pl.pallas_call(
        _kernel,
        in_specs=[hbm] * 6 + [pl.BlockSpec(memory_space=pltpu.VMEM)] + [hbm] * 3,
        out_specs=hbm,
        out_shape=jax.ShapeDtypeStruct((S, M), BF),
        scratch_shapes=[
            pltpu.VMEM((S, M), BF), pltpu.VMEM((S, DC), BF),
            pltpu.VMEM((S, M), BF), pltpu.VMEM((S, M), F32),
            pltpu.VMEM((7, S // 2, KH), BF), pltpu.VMEM((7, S // 2, KH), BF),
            pltpu.VMEM((2, M, 8, D), U32), pltpu.VMEM((2, DC, 8, D), U32), pltpu.VMEM((2, DC, 8, D), U32),
            pltpu.VMEM((H * D, M), BF),
            pltpu.VMEM((7, KH, D), BF), pltpu.VMEM((M - 2 * KH, 2 * D), BF),
            pltpu.VMEM((7, KH, 2 * D), BF),
            pltpu.VMEM((2, S, D), BF), pltpu.VMEM((2, S, D), BF), pltpu.VMEM((2, S, D), BF),
            pltpu.VMEM((F, M), BF), pltpu.VMEM((F, M), BF), pltpu.VMEM((F, M), BF),
            pltpu.VMEM((NR, 8, 128), F32),
            pltpu.SemaphoreType.DMA((NR,)), pltpu.SemaphoreType.DMA((NR,)),
            pltpu.SemaphoreType.DMA((12,)), pltpu.SemaphoreType.DMA((5,)),
            pltpu.SemaphoreType.DMA((NR,)),
        ],
        compiler_params=pltpu.CompilerParams(vmem_limit_bytes=120 * 1024 * 1024),
    )(A_x.reshape(S, M), A_c_kv.reshape(S, DC), A_w_q, A_w_uk, A_w_uv, A_w_o.reshape(H * D, M),
      B_w_r, B_w_gate.T, B_w_up.T, B_w_down)
    return out.reshape(1, S, M)
```

```python
import jax
import jax.numpy as jnp
import numpy as np
from jax import lax
import jax.experimental.pallas as pl
import jax.experimental.pallas.tpu as pltpu

S, M, DC, H, D, F, C = 2048, 640, 512, 32, 128, 1728, 8
NP = H // 2
BQ = 128
RB = 2 * BQ
NR = S // RB
KH = 256
AHEAD = 4
QSCALE = float(D ** -0.5) * 1.4426950408889634
EPS_BF = float(np.asarray(1e-5, dtype=jnp.bfloat16))
NEG = -1e30
BF = jnp.bfloat16
F32 = jnp.float32
I32 = jnp.int32
U32 = jnp.uint32


def _rb(v):
    return v.astype(BF).astype(F32)


def _dot(a, b):
    return jnp.dot(a, b, preferred_element_type=F32)


def _dot_nt(a, b):
    return lax.dot_general(a, b, (((1,), (1,)), ((), ())), preferred_element_type=F32)


def _ds(start, size, align):
    if isinstance(start, int):
        return pl.ds(start, size)
    return pl.ds(pl.multiple_of(start, align), size)


def _left7(a11, a12, a21, a22):
    return [a11 + a22, a21 + a22, a11, a22, a11 + a12, a21 - a11, a12 - a22]


def _right7(b11, b12, b21, b22):
    return [b11 + b22, b11, b12 - b22, b21 - b11, b22, b11 + b12, b21 + b22]


def _block_matmul(a, b):
    def m(i):
        return _dot(a(i), b(i))

    m4 = m(3)
    m3 = m(2)
    m1 = m(0)
    c11 = m1 + m4
    c22 = m1 + m3
    m2 = m(1)
    c21 = m2 + m4
    c22 = c22 - m2
    m5 = m(4)
    c12 = m3 + m5
    c11 = c11 - m5
    c22 = c22 + m(5)
    c11 = c11 + m(6)
    return c11, c12, c21, c22


def _attention(q_s, k_s, v_s, lag, fill):
    nb = S // BQ
    look = 2
    row = lax.broadcasted_iota(I32, (BQ, BQ), 0)
    col = lax.broadcasted_iota(I32, (BQ, BQ), 1)
    tri = col <= row
    sums = []

    def qk(h, i):
        return _dot_nt(q_s[h, i * BQ:(i + 1) * BQ, :], k_s[h, 0:(i + 1) * BQ, :])

    def softmax_pv(h, i, s):
        sd = jnp.where(tri, s[:, i * BQ:], NEG)
        s = jnp.concatenate([s[:, :i * BQ], sd], axis=1) if i > 0 else sd
        m = jnp.max(s, axis=1, keepdims=True)
        if len(sums) >= lag:
            old = sums.pop(0)
            m = jnp.where(old < 0.0, old, m)
        p = jnp.exp2(s - m)
        l = jnp.sum(p, axis=1, keepdims=True)
        sums.append(l)
        o = _dot(p.astype(BF), v_s[h, 0:(i + 1) * BQ, :])
        r = pl.reciprocal(l, approx=True)
        r = r * (2.0 - l * r)
        return o * r

    order = list(range(0, nb, 2)) + list(range(nb - 1, 0, -2))
    items = [(h, i) for h in range(2) for i in order]
    scores, ctx = {}, {}
    for t in range(look):
        scores[t] = qk(*items[t])
    for t, it in enumerate(items):
        if t + look < len(items):
            scores[t + look] = qk(*items[t + look])
        fill(t)
        ctx[it] = softmax_pv(*it, scores.pop(t))
    return ctx


def _kernel(x_hbm, c_hbm, wq_hbm, wk_hbm, wv_hbm, wo_hbm, wr_ref, wg_hbm, wu_hbm, wd_hbm, o_hbm,
            x_s, c_s, xn_s, acc_s, xa_s, ca_s, wq3, wk3, wv3, wo_s, wq_s, wqt_s, wkv_s, q_s, k_s, v_s,
            wg_s, wu_s, wd_s, r_s, sem_x, sem_c, sem_w, sem_f, sem_o):

    w3 = [(wk_hbm.bitcast(U32), wk3), (wv_hbm.bitcast(U32), wv3), (wq_hbm.bitcast(U32), wq3)]

    def w_copies(k, lo, hi):
        return [pltpu.make_async_copy(src.at[:, lo:hi, :], dst.at[lo // 4, :, lo % 4:lo % 4 + hi - lo, :],
                                      sem_w.at[3 * k + i])
                for i, (src, dst) in enumerate(w3)]

    w_first, w_a, w_b = w_copies(0, 0, 1), w_copies(1, 1, 4), w_copies(2, 4, 8)
    w_c = w_copies(3, 8, 12) + w_copies(4, 12, 16)
    wo_first = pltpu.make_async_copy(wo_hbm.at[0:2 * D, :], wo_s.at[0:2 * D, :], sem_f.at[3])
    wo_rest = pltpu.make_async_copy(wo_hbm.at[2 * D:H * D, :], wo_s.at[2 * D:H * D, :], sem_f.at[4])
    f_copies = [pltpu.make_async_copy(wg_hbm, wg_s, sem_f.at[0]),
                pltpu.make_async_copy(wu_hbm, wu_s, sem_f.at[1]),
                pltpu.make_async_copy(wd_hbm, wd_s, sem_f.at[2])]

    def in_copies(r):
        rows = _ds(r * RB, RB, RB)
        return [pltpu.make_async_copy(c_hbm.at[rows, :], c_s.at[rows, :], sem_c.at[r]),
                pltpu.make_async_copy(x_hbm.at[rows, :], x_s.at[rows, :], sem_x.at[r])]

    def start(copies):
        for cp in copies:
            cp.start()

    def wait(copies):
        for cp in copies:
            cp.wait()

    def pick(w, p):
        n = w.shape[1]
        u = w.reshape(4 * n * 8, D)[pl.ds((p // 4) * (n * 8) + p % 4, n, stride=8), :]
        return pltpu.bitcast(u << 16, F32), pltpu.bitcast((u >> 16) << 16, F32)

    def load_wkv(p):
        wk = jnp.concatenate(pick(wk3, p), axis=1)
        wv = jnp.concatenate(pick(wv3, p), axis=1)
        for i, b in enumerate(_right7(wk[:KH], wv[:KH], wk[KH:], wv[KH:])):
            wkv_s[i] = b.astype(BF)

    def load_wq(p):
        h0, h1 = pick(wq3, p)
        for i, b in enumerate(_right7(h0[:KH], h1[:KH], h0[KH:2 * KH], h1[KH:2 * KH])):
            wq_s[i] = b.astype(BF)
        wqt_s[...] = jnp.concatenate([h0[2 * KH:], h1[2 * KH:]], axis=1).astype(BF)

    def kv_proj(r, n, direct=None):
        rows = _ds(r * BQ, n * BQ, BQ)
        c4 = _block_matmul(lambda i: direct[i] if direct and i in direct else ca_s[i, rows, :],
                           lambda i: wkv_s[i])
        for t in range(n):
            for u in range(2):
                dst = _ds((r + t) * RB + u * BQ, BQ, BQ)
                for h in range(2):
                    k_s[h, dst, :] = c4[2 * u][t * BQ:(t + 1) * BQ, h * D:(h + 1) * D].astype(BF)
                    v_s[h, dst, :] = c4[2 * u + 1][t * BQ:(t + 1) * BQ, h * D:(h + 1) * D].astype(BF)

    def q_proj(r, n):
        rows = _ds(r * BQ, n * BQ, BQ)
        c4 = _block_matmul(lambda i: xa_s[i, rows, :], lambda i: wq_s[i])
        rest = _dot(xn_s[_ds(r * RB, n * RB, RB), 2 * KH:], wqt_s[...])
        for t in range(n):
            for u in range(2):
                dst = _ds((r + t) * RB + u * BQ, BQ, BQ)
                lo = t * RB + u * BQ
                for h in range(2):
                    q = c4[2 * u + h][t * BQ:(t + 1) * BQ] + rest[lo:lo + BQ, h * D:(h + 1) * D]
                    q_s[h, dst, :] = (q * QSCALE).astype(BF)

    def o_proj(p, ctx, n, emit):
        wo = wo_s[_ds(p * 2 * D, 2 * D, 2 * D), :]
        wf = wo.astype(F32)
        b7 = [b.astype(BF) for b in _right7(wf[:D, :KH], wf[:D, KH:2 * KH], wf[D:, :KH], wf[D:, KH:2 * KH])]
        for r in range(0, NR, n):
            full = jnp.concatenate(
                [jnp.concatenate([ctx[0, i], ctx[1, i]], axis=1).astype(BF) for i in range(2 * r, 2 * (r + n))],
                axis=0)
            a7 = [_left7(ctx[0, 2 * t], ctx[1, 2 * t], ctx[0, 2 * t + 1], ctx[1, 2 * t + 1])
                  for t in range(r, r + n)]
            c4 = _block_matmul(lambda i: jnp.concatenate([a[i].astype(BF) for a in a7], axis=0),
                               lambda i: b7[i])
            rest = _dot(full, wo[:, 2 * KH:])
            left = jnp.concatenate(
                [jnp.concatenate([c4[2 * u][t * BQ:(t + 1) * BQ], c4[2 * u + 1][t * BQ:(t + 1) * BQ]], axis=1)
                 for t in range(n) for u in range(2)], axis=0)
            emit(r, jnp.concatenate([left, rest], axis=1))

    start(w_first[:2])
    start(in_copies(0))
    start(w_first[2:])
    wait(w_first)
    for r in range(1, AHEAD):
        start(in_copies(r))
    load_wkv(0)
    load_wq(0)

    def prologue(r, carry):
        @pl.when(r + AHEAD < NR)
        def _():
            start(in_copies(jnp.minimum(r + AHEAD, NR - 1)))

        @pl.when(r == NR - AHEAD - 1)
        def _():
            start(w_a + [wo_first])

        wait(in_copies(r))
        rows, half = _ds(r * RB, RB, RB), _ds(r * BQ, BQ, BQ)
        cb = c_s[rows, :]
        c = cb.astype(F32)
        for i, a in enumerate(_left7(c[:BQ, :KH], c[:BQ, KH:], c[BQ:, :KH], c[BQ:, KH:])):
            ca_s[i, half, :] = a.astype(BF)
        kv_proj(r, 1, {2: cb[:BQ, :KH], 3: cb[BQ:, KH:]})

        x = x_s[rows, :].astype(F32)
        mean = jnp.sum(x, axis=1, keepdims=True) / M
        cen = x - mean
        var = jnp.sum(cen * cen, axis=1, keepdims=True) / M
        den = _rb(jnp.sqrt(_rb(_rb(var) + EPS_BF)))
        xn = (_rb(x - _rb(mean)) * (1.0 / den)).astype(BF)
        xn_s[rows, :] = xn
        xf = xn.astype(F32)
        acc_s[rows, :] = x + xf
        for i, a in enumerate(_left7(xf[:BQ, :KH], xf[:BQ, KH:2 * KH], xf[BQ:, :KH], xf[BQ:, KH:2 * KH])):
            xa_s[i, half, :] = a.astype(BF)

        sc = jnp.sum(xf * wr_ref[...].reshape(1, M).astype(F32), axis=1, keepdims=True)
        lane = lax.broadcasted_iota(I32, (8, 128), 1)
        dense = jnp.full((8, 128), -jnp.inf, F32)
        for i in range(RB // 8):
            dense = jnp.where(lane == i, sc[i * 8:(i + 1) * 8, :], dense)
        r_s[r] = dense
        q_proj(r, 1)
        return carry

    lax.fori_loop(0, NR, prologue, 0)
    wait(w_a)
    start(w_b + [wo_rest])
    load_wq(1)
    wait([wo_first])

    def accumulate(r, out):
        acc_s[r * RB:r * RB + out.shape[0], :] += out

    def body(p, carry):
        @pl.when(p == 1)
        def _():
            wait(w_b + [wo_rest])
            start(w_c + f_copies)

        @pl.when(p == 4)
        def _():
            wait(w_c + f_copies)

        ctx = _attention(q_s, k_s, v_s, 10, lambda t: None)
        for r in range(0, NR, 4):
            q_proj(r, 4)
        load_wq(jnp.minimum(p + 2, NP - 1))
        load_wkv(p + 1)
        for r in range(0, NR, 2):
            kv_proj(r, 2)
        o_proj(p, ctx, 4, accumulate)
        return carry

    lax.fori_loop(0, NP - 1, body, 0)

    shp = (NR * 8, 128)
    sc = _rb(r_s[...].reshape(shp))
    sc = jnp.where(sc != sc, -jnp.inf, sc)
    sub = lax.broadcasted_iota(I32, shp, 0)
    lane = lax.broadcasted_iota(I32, shp, 1)
    tok = jnp.where(lane < RB // 8, (sub // 8) * RB + lane * 8 + sub % 8, S)
    slot = lax.broadcasted_iota(I32, (C, 1), 0)
    row16 = lax.broadcasted_iota(I32, (16, 1), 0)
    xsel = jnp.zeros((C, M), F32)
    rsel = jnp.zeros((C, 1), F32)
    idxs = []
    for j in range(C):
        mx = jnp.max(sc)
        idx = jnp.min(jnp.where(sc == mx, tok, S))
        hit = tok == idx
        sc = jnp.where(hit, -jnp.inf, sc)
        tok = jnp.where(hit, S, tok)
        idx = jnp.clip(idx, 0, S - 1)
        idxs.append(idx)
        blk = xn_s[_ds((idx // 16) * 16, 16, 16), :].astype(F32)
        xrow = jnp.sum(jnp.where(row16 == idx % 16, blk, 0.0), axis=0, keepdims=True)
        xsel = jnp.where(slot == j, xrow, xsel)
        rsel = jnp.where(slot == j, mx, rsel)
    xs = jnp.concatenate([xsel, jnp.zeros((16 - C, M), F32)], axis=0).astype(BF)

    nf = pl.cdiv(F, D)
    first = 8
    st = {"y": None}

    def ffn(t):
        j, second = divmod(t - first, 2)
        if not 0 <= j <= nf:
            return
        cols = slice(j * D, min((j + 1) * D, F))
        if not second:
            if j < nf:
                st["g"] = _dot_nt(xs, wg_s[cols, :])
            if j > 0:
                part = _dot(st.pop("h"), wd_s[(j - 1) * D:min(j * D, F), :])
                st["y"] = part if st["y"] is None else st["y"] + part
        elif j < nf:
            g = st.pop("g")
            st["h"] = (g * jax.nn.sigmoid(g) * _dot_nt(xs, wu_s[cols, :])).astype(BF)

    ctx = _attention(q_s, k_s, v_s, 11, ffn)
    for t in range(len(ctx), first + 2 * nf + 1):
        ffn(t)
    y = st["y"][:C] * jax.nn.sigmoid(rsel)
    for j in range(C):
        rows = _ds((idxs[j] // 8) * 8, 8, 8)
        acc_s[rows, :] += jnp.where(slot == idxs[j] % 8, y[j:j + 1, :], 0.0)

    outs = []

    def emit(r, out):
        rows = pl.ds(r * RB, RB)
        x_s[rows, :] = (acc_s[rows, :] + out).astype(BF)
        outs.append(pltpu.make_async_copy(x_s.at[rows, :], o_hbm.at[rows, :], sem_o.at[r]))
        outs[-1].start()

    o_proj(NP - 1, ctx, 1, emit)
    wait(outs)


@jax.jit
def pallas_parallel_sum__compressed_kv_cla__moe_arch_mod__prompt_kernel(
    A_x: jax.Array,
    A_c_kv: jax.Array,
    A_w_q: jax.Array,
    A_w_uk: jax.Array,
    A_w_uv: jax.Array,
    A_w_o: jax.Array,
    B_x: jax.Array,
    B_w_r: jax.Array,
    B_w_gate: jax.Array,
    B_w_up: jax.Array,
    B_w_down: jax.Array,
):
    del B_x
    hbm = pl.BlockSpec(memory_space=pltpu.HBM)
    out = pl.pallas_call(
        _kernel,
        in_specs=[hbm] * 6 + [pl.BlockSpec(memory_space=pltpu.VMEM)] + [hbm] * 3,
        out_specs=hbm,
        out_shape=jax.ShapeDtypeStruct((S, M), BF),
        scratch_shapes=[
            pltpu.VMEM((S, M), BF), pltpu.VMEM((S, DC), BF),
            pltpu.VMEM((S, M), BF), pltpu.VMEM((S, M), F32),
            pltpu.VMEM((7, S // 2, KH), BF), pltpu.VMEM((7, S // 2, KH), BF),
            pltpu.VMEM((4, M, 8, D), U32), pltpu.VMEM((4, DC, 8, D), U32), pltpu.VMEM((4, DC, 8, D), U32),
            pltpu.VMEM((H * D, M), BF),
            pltpu.VMEM((7, KH, D), BF), pltpu.VMEM((M - 2 * KH, 2 * D), BF),
            pltpu.VMEM((7, KH, 2 * D), BF),
            pltpu.VMEM((2, S, D), BF), pltpu.VMEM((2, S, D), BF), pltpu.VMEM((2, S, D), BF),
            pltpu.VMEM((F, M), BF), pltpu.VMEM((F, M), BF), pltpu.VMEM((F, M), BF),
            pltpu.VMEM((NR, 8, 128), F32),
            pltpu.SemaphoreType.DMA((NR,)), pltpu.SemaphoreType.DMA((NR,)),
            pltpu.SemaphoreType.DMA((15,)), pltpu.SemaphoreType.DMA((5,)),
            pltpu.SemaphoreType.DMA((NR,)),
        ],
        compiler_params=pltpu.CompilerParams(vmem_limit_bytes=120 * 1024 * 1024),
    )(A_x.reshape(S, M), A_c_kv.reshape(S, DC), A_w_q, A_w_uk, A_w_uv, A_w_o.reshape(H * D, M),
      B_w_r, B_w_gate.T, B_w_up.T, B_w_down)
    return out.reshape(1, S, M)
```

```python
import jax
import jax.numpy as jnp
import numpy as np
from jax import lax
import jax.experimental.pallas as pl
import jax.experimental.pallas.tpu as pltpu

S, M, DC, H, D, F, C = 2048, 640, 512, 32, 128, 1728, 8
NP = H // 2
BQ = 128
RB = 256
NR = S // RB
AHEAD = 4
QB, KB, OB = 1024, 1024, 2048
FFN_AT = 8
QSCALE = float(D ** -0.5) * 1.4426950408889634
EPS_BF = float(np.asarray(1e-5, dtype=jnp.bfloat16))
NEG = -1e30
BF = jnp.bfloat16
F32 = jnp.float32
I32 = jnp.int32
U32 = jnp.uint32


def _rb(v):
    return v.astype(BF).astype(F32)


def _dot(a, b):
    return jnp.dot(a, b, preferred_element_type=F32)


def _dot_nt(a, b):
    return lax.dot_general(a, b, (((1,), (1,)), ((), ())), preferred_element_type=F32)


def _ds(start, size, align):
    if isinstance(start, int):
        return pl.ds(start, size)
    return pl.ds(pl.multiple_of(start, align), size)


def _attention(q_s, k_s, v_s, fill):
    nb = S // BQ
    look = 2
    row = lax.broadcasted_iota(I32, (BQ, BQ), 0)
    col = lax.broadcasted_iota(I32, (BQ, BQ), 1)
    tri = col <= row

    def qk(h, i):
        return _dot_nt(q_s[h, i * BQ:(i + 1) * BQ, :], k_s[h, 0:(i + 1) * BQ, :])

    def softmax_pv(h, i, s):
        sd = jnp.where(tri, s[:, i * BQ:], NEG)
        s = jnp.concatenate([s[:, :i * BQ], sd], axis=1) if i > 0 else sd
        m = jnp.max(s, axis=1, keepdims=True)
        p = jnp.exp2(s - m)
        l = jnp.sum(p, axis=1, keepdims=True)
        o = _dot(p.astype(BF), v_s[h, 0:(i + 1) * BQ, :])
        r = pl.reciprocal(l, approx=True)
        r = r * (2.0 - l * r)
        return (o * r).astype(BF)

    order = list(range(0, nb, 2)) + list(range(nb - 1, 0, -2))
    items = [(h, i) for h in range(2) for i in order]
    scores, ctx = {}, {}
    for t in range(look):
        scores[t] = qk(*items[t])
    for t, it in enumerate(items):
        if t + look < len(items):
            scores[t + look] = qk(*items[t + look])
        fill(t)
        ctx[it] = softmax_pv(*it, scores.pop(t))
    return ctx


def _kernel(x_hbm, c_hbm, wq_hbm, wk_hbm, wv_hbm, wo_hbm, wr_ref, wg_hbm, wu_hbm, wd_hbm, o_hbm,
            x_s, c_s, xn_s, acc_s, wq3, wk3, wv3, wo_s, wq_s, wkv_s, q_s, k_s, v_s,
            wg_s, wu_s, wd_s, r_s, sem_x, sem_c, sem_w, sem_f, sem_o):

    w3 = [(wk_hbm.bitcast(U32), wk3), (wv_hbm.bitcast(U32), wv3), (wq_hbm.bitcast(U32), wq3)]

    def w_copies(k, lo, hi):
        return [pltpu.make_async_copy(src.at[:, lo:hi, :], dst.at[lo // 4, :, lo % 4:lo % 4 + hi - lo, :],
                                      sem_w.at[3 * k + i])
                for i, (src, dst) in enumerate(w3)]

    w_first, w_a, w_b = w_copies(0, 0, 1), w_copies(1, 1, 4), w_copies(2, 4, 8)
    w_c = w_copies(3, 8, 12) + w_copies(4, 12, 16)
    wo_first = pltpu.make_async_copy(wo_hbm.at[0:2 * D, :], wo_s.at[0:2 * D, :], sem_f.at[3])
    wo_rest = pltpu.make_async_copy(wo_hbm.at[2 * D:H * D, :], wo_s.at[2 * D:H * D, :], sem_f.at[4])
    f_copies = [pltpu.make_async_copy(wg_hbm, wg_s, sem_f.at[0]),
                pltpu.make_async_copy(wu_hbm, wu_s, sem_f.at[1]),
                pltpu.make_async_copy(wd_hbm, wd_s, sem_f.at[2])]

    def in_copies(r):
        rows = _ds(r * RB, RB, RB)
        return [pltpu.make_async_copy(c_hbm.at[rows, :], c_s.at[rows, :], sem_c.at[r]),
                pltpu.make_async_copy(x_hbm.at[rows, :], x_s.at[rows, :], sem_x.at[r])]

    def start(copies):
        for cp in copies:
            cp.start()

    def wait(copies):
        for cp in copies:
            cp.wait()

    def pick(w, p):
        n = w.shape[1]
        u = w.reshape(4 * n * 8, D)[pl.ds((p // 4) * (n * 8) + p % 4, n, stride=8), :]
        return jnp.concatenate([pltpu.bitcast(u << 16, F32).astype(BF),
                                pltpu.bitcast((u >> 16) << 16, F32).astype(BF)], axis=1)

    def load_wkv(p):
        wkv_s[:, 0:2 * D] = pick(wk3, p)
        wkv_s[:, 2 * D:4 * D] = pick(wv3, p)

    def load_wq(p):
        wq_s[...] = pick(wq3, p)

    def kv_proj(rows):
        kv = _dot(c_s[rows, :], wkv_s[...]).astype(BF)
        for h in range(2):
            k_s[h, rows, :] = kv[:, h * D:(h + 1) * D]
            v_s[h, rows, :] = kv[:, (2 + h) * D:(3 + h) * D]

    def q_proj(rows):
        q = (_dot(xn_s[rows, :], wq_s[...]) * QSCALE).astype(BF)
        for h in range(2):
            q_s[h, rows, :] = q[:, h * D:(h + 1) * D]

    def o_proj(p, ctx, step, emit):
        wo = wo_s[_ds(p * 2 * D, 2 * D, 2 * D), :]
        for r in range(0, S, step):
            a = jnp.concatenate([jnp.concatenate([ctx[0, i], ctx[1, i]], axis=1)
                                 for i in range(r // BQ, (r + step) // BQ)], axis=0)
            emit(r, _dot(a, wo))

    start(w_first[:2])
    start(in_copies(0))
    start(w_first[2:])
    wait(w_first)
    for r in range(1, AHEAD):
        start(in_copies(r))
    load_wkv(0)
    load_wq(0)

    def prologue(r, carry):
        @pl.when(r + AHEAD < NR)
        def _():
            start(in_copies(jnp.minimum(r + AHEAD, NR - 1)))

        @pl.when(r == NR - AHEAD - 1)
        def _():
            start(w_a + [wo_first])

        wait(in_copies(r))
        rows = _ds(r * RB, RB, RB)
        kv_proj(rows)

        x = x_s[rows, :].astype(F32)
        mean = jnp.sum(x, axis=1, keepdims=True) / M
        cen = x - mean
        var = jnp.sum(cen * cen, axis=1, keepdims=True) / M
        den = _rb(jnp.sqrt(_rb(_rb(var) + EPS_BF)))
        xn = (_rb(x - _rb(mean)) * (1.0 / den)).astype(BF)
        xn_s[rows, :] = xn
        xf = xn.astype(F32)
        acc_s[rows, :] = x + xf

        sc = jnp.sum(xf * wr_ref[...].reshape(1, M).astype(F32), axis=1, keepdims=True)
        lane = lax.broadcasted_iota(I32, (8, 128), 1)
        dense = jnp.full((8, 128), -jnp.inf, F32)
        for i in range(RB // 8):
            dense = jnp.where(lane == i, sc[i * 8:(i + 1) * 8, :], dense)
        r_s[r] = dense
        q_proj(rows)
        return carry

    lax.fori_loop(0, NR, prologue, 0)
    wait(w_a)
    start(w_b + [wo_rest])
    load_wq(1)
    wait([wo_first])

    def accumulate(r, out):
        acc_s[r:r + out.shape[0], :] += out

    def body(p, carry):
        @pl.when(p == 1)
        def _():
            wait(w_b + [wo_rest])
            start(w_c + f_copies)

        @pl.when(p == 4)
        def _():
            wait(w_c + f_copies)

        ctx = _attention(q_s, k_s, v_s, lambda t: None)
        for r in range(0, S, QB):
            q_proj(pl.ds(r, QB))
        load_wq(jnp.minimum(p + 2, NP - 1))
        load_wkv(p + 1)
        for r in range(0, S, KB):
            kv_proj(pl.ds(r, KB))
        o_proj(p, ctx, OB, accumulate)
        return carry

    lax.fori_loop(0, NP - 1, body, 0)

    shp = (NR * 8, 128)
    sc = _rb(r_s[...].reshape(shp))
    sc = jnp.where(sc != sc, -jnp.inf, sc)
    sub = lax.broadcasted_iota(I32, shp, 0)
    lane = lax.broadcasted_iota(I32, shp, 1)
    tok = jnp.where(lane < RB // 8, (sub // 8) * RB + lane * 8 + sub % 8, S)
    slot = lax.broadcasted_iota(I32, (C, 1), 0)
    row16 = lax.broadcasted_iota(I32, (16, 1), 0)
    xsel = jnp.zeros((C, M), F32)
    rsel = jnp.zeros((C, 1), F32)
    idxs = []
    for j in range(C):
        mx = jnp.max(sc)
        idx = jnp.min(jnp.where(sc == mx, tok, S))
        hit = tok == idx
        sc = jnp.where(hit, -jnp.inf, sc)
        tok = jnp.where(hit, S, tok)
        idx = jnp.clip(idx, 0, S - 1)
        idxs.append(idx)
        blk = xn_s[_ds((idx // 16) * 16, 16, 16), :].astype(F32)
        xrow = jnp.sum(jnp.where(row16 == idx % 16, blk, 0.0), axis=0, keepdims=True)
        xsel = jnp.where(slot == j, xrow, xsel)
        rsel = jnp.where(slot == j, mx, rsel)
    xs = jnp.concatenate([xsel, jnp.zeros((16 - C, M), F32)], axis=0).astype(BF)

    nf = pl.cdiv(F, D)
    first = FFN_AT
    st = {"y": None}

    def ffn(t):
        j, second = divmod(t - first, 2)
        if not 0 <= j <= nf:
            return
        cols = slice(j * D, min((j + 1) * D, F))
        if not second:
            if j < nf:
                st["g"] = _dot_nt(xs, wg_s[cols, :])
            if j > 0:
                part = _dot(st.pop("h"), wd_s[(j - 1) * D:min(j * D, F), :])
                st["y"] = part if st["y"] is None else st["y"] + part
        elif j < nf:
            g = st.pop("g")
            st["h"] = (g * jax.nn.sigmoid(g) * _dot_nt(xs, wu_s[cols, :])).astype(BF)

    ctx = _attention(q_s, k_s, v_s, ffn)
    for t in range(len(ctx), first + 2 * nf + 1):
        ffn(t)
    y = st["y"][:C] * jax.nn.sigmoid(rsel)
    for j in range(C):
        rows = _ds((idxs[j] // 8) * 8, 8, 8)
        acc_s[rows, :] += jnp.where(slot == idxs[j] % 8, y[j:j + 1, :], 0.0)

    outs = []

    def emit(r, out):
        rows = pl.ds(r, RB)
        x_s[rows, :] = (acc_s[rows, :] + out).astype(BF)
        outs.append(pltpu.make_async_copy(x_s.at[rows, :], o_hbm.at[rows, :], sem_o.at[r // RB]))
        outs[-1].start()

    o_proj(NP - 1, ctx, RB, emit)
    wait(outs)


@jax.jit
def pallas_parallel_sum__compressed_kv_cla__moe_arch_mod__prompt_kernel(
    A_x: jax.Array,
    A_c_kv: jax.Array,
    A_w_q: jax.Array,
    A_w_uk: jax.Array,
    A_w_uv: jax.Array,
    A_w_o: jax.Array,
    B_x: jax.Array,
    B_w_r: jax.Array,
    B_w_gate: jax.Array,
    B_w_up: jax.Array,
    B_w_down: jax.Array,
):
    del B_x
    hbm = pl.BlockSpec(memory_space=pltpu.HBM)
    out = pl.pallas_call(
        _kernel,
        in_specs=[hbm] * 6 + [pl.BlockSpec(memory_space=pltpu.VMEM)] + [hbm] * 3,
        out_specs=hbm,
        out_shape=jax.ShapeDtypeStruct((S, M), BF),
        scratch_shapes=[
            pltpu.VMEM((S, M), BF), pltpu.VMEM((S, DC), BF),
            pltpu.VMEM((S, M), BF), pltpu.VMEM((S, M), F32),
            pltpu.VMEM((4, M, 8, D), U32), pltpu.VMEM((4, DC, 8, D), U32), pltpu.VMEM((4, DC, 8, D), U32),
            pltpu.VMEM((H * D, M), BF),
            pltpu.VMEM((M, 2 * D), BF), pltpu.VMEM((DC, 4 * D), BF),
            pltpu.VMEM((2, S, D), BF), pltpu.VMEM((2, S, D), BF), pltpu.VMEM((2, S, D), BF),
            pltpu.VMEM((F, M), BF), pltpu.VMEM((F, M), BF), pltpu.VMEM((F, M), BF),
            pltpu.VMEM((NR, 8, 128), F32),
            pltpu.SemaphoreType.DMA((NR,)), pltpu.SemaphoreType.DMA((NR,)),
            pltpu.SemaphoreType.DMA((15,)), pltpu.SemaphoreType.DMA((5,)),
            pltpu.SemaphoreType.DMA((NR,)),
        ],
        compiler_params=pltpu.CompilerParams(vmem_limit_bytes=120 * 1024 * 1024),
    )(A_x.reshape(S, M), A_c_kv.reshape(S, DC), A_w_q, A_w_uk, A_w_uv, A_w_o.reshape(H * D, M),
      B_w_r, B_w_gate.T, B_w_up.T, B_w_down)
    return out.reshape(1, S, M)
```
